```python
import jax
import jax.numpy as jnp

def _softmax(x, axis=-1):
    return jax.nn.softmax(x, axis=axis)

def _gelu(x):
    return jax.nn.gelu(x, approximate=True)

def _silu(x):
    return jax.nn.silu(x)

def _sigmoid(x):
    return jax.nn.sigmoid(x)

def _layernorm(x, axis=-1, eps=1e-05):
    m = jnp.mean(x, axis=axis, keepdims=True)
    v = jnp.var(x, axis=axis, keepdims=True)
    return (x - m) / jnp.sqrt(v + eps)

def _scatter_add(tgt, idx, src, axis=0):
    return tgt.at[idx].add(src)

def _segment_sum(src, seg, n):
    return jax.ops.segment_sum(src, seg, n)

class _Rng:

    def __init__(self, key):
        self._k = key

    def _next(self):
        self._k, sub = jax.random.split(self._k)
        return sub

    def normal(self, shape):
        return jax.random.normal(self._next(), shape, dtype=jnp.bfloat16)

    def randint(self, lo, hi, shape):
        return jax.random.randint(self._next(), shape, lo, hi, dtype=jnp.int32)

    def uniform(self, shape, lo=0.0, hi=1.0):
        return jax.random.uniform(self._next(), shape, jnp.bfloat16, lo, hi)

    def permutation(self, n):
        return jax.random.permutation(self._next(), n)
kernel_name = 'concat_heads__sliding_local_dilated__memory_aug_recurrent_mem_tr__prompt'

def setup_inputs():
    _rng = _Rng(jax.random.key(int.from_bytes(__import__("os").urandom(4), "little")))
    _w = lambda a: (lambda t: t.astype(jnp.bfloat16) if jnp.issubdtype(t.dtype, jnp.floating) else t)(jnp.asarray(a))

    def _A_setup():
        B, S, D = (1, 2048, 640)
        return {'x': _w((lambda *s: _rng.normal(s) * 0.05)(B, S, D)), 'wqkv': _w((lambda *s: _rng.normal(s) * 0.05)(D, 3 * D)), 'wo': _w((lambda *s: _rng.normal(s) * 0.05)(D, D))}
    _A_in = _A_setup()

    def _B_setup():
        B, S, Dm = (1, 2048, 640)
        H, Dh = (32, 192)
        M, seg = (8, 32)
        seg = min(seg, S)
        S = S // seg * seg
        return {'x': _w((lambda *s: _rng.normal(s) * 0.05)(B, S, Dm)), 'mem0': _w((lambda *s: _rng.normal(s) * 0.05)(B, M, Dm)), 'Wq': _w((lambda *s: _rng.normal(s) * 0.05)(Dm, H, Dh) * Dm ** (-0.5)), 'Wk': _w((lambda *s: _rng.normal(s) * 0.05)(Dm, H, Dh) * Dm ** (-0.5)), 'Wv': _w((lambda *s: _rng.normal(s) * 0.05)(Dm, H, Dh) * Dm ** (-0.5)), 'Wo': _w((lambda *s: _rng.normal(s) * 0.05)(H, Dh, Dm) * (H * Dh) ** (-0.5)), 'seg_len': seg}
    _B_in = _B_setup()
    return {'A_x': _A_in['x'], 'A_wqkv': _A_in['wqkv'], 'A_wo': _A_in['wo'], 'B_x': _B_in['x'], 'B_mem0': _B_in['mem0'], 'B_Wq': _B_in['Wq'], 'B_Wk': _B_in['Wk'], 'B_Wv': _B_in['Wv'], 'B_Wo': _B_in['Wo'], 'B_seg_len': _B_in['seg_len']}

def reference(A_x, A_wqkv, A_wo, B_x, B_mem0, B_Wq, B_Wk, B_Wv, B_Wo, B_seg_len):

    def _A_ref(x, wqkv, wo):
        B, S, D = x.shape
        H = 32
        Dh = D // H
        W, dil = (8, 2)
        qkv = (lambda x, *d: x.transpose(*d))((x @ wqkv).reshape(B, S, 3, H, Dh), 2, 0, 3, 1, 4)
        q, k, v = (qkv[0], qkv[1], qkv[2])
        scale = Dh ** (-0.5)
        pos = jnp.arange(S)
        off = jnp.arange(W) * dil
        idx = pos[:, None] - off[None, :]
        mask = idx >= 0
        idx_c = jnp.where(mask, idx, 0).reshape(-1)
        kg = k[:, :, idx_c, :].reshape(B, H, S, W, Dh)
        vg = v[:, :, idx_c, :].reshape(B, H, S, W, Dh)
        logits = jnp.einsum('bhsd,bhswd->bhsw', q, kg) * scale
        logits = jnp.where(mask[None, None, :, :], logits, -1000000000.0)
        attn = _softmax(logits, axis=-1)
        o = jnp.einsum('bhsw,bhswd->bhsd', attn, vg)
        return (lambda x, *d: x.transpose(*d))(o, 0, 2, 1, 3).reshape(B, S, D) @ wo

    def _B_ref(x, mem0, Wq, Wk, Wv, Wo, seg_len):
        B, S, Dm = x.shape
        H, Dh = (Wq.shape[1], Wq.shape[2])
        M = mem0.shape[1]
        scale = Dh ** (-0.5)
        n_seg = S // seg_len
        L = M + seg_len
        idx = jnp.arange(L)
        mask = (idx[:, None] < M) | (idx[:, None] >= idx[None, :])
        mem = mem0
        outs = []
        for s in range(n_seg):
            xs = x[:, s * seg_len:(s + 1) * seg_len, :].copy()
            h = jnp.concatenate([mem, xs], axis=1)
            q = jnp.einsum('btd,dhe->bhte', h, Wq)
            k = jnp.einsum('btd,dhe->bhte', h, Wk)
            v = jnp.einsum('btd,dhe->bhte', h, Wv)
            scores = jnp.einsum('bhqe,bhke->bhqk', q, k) * scale
            scores = jnp.where(mask[None, None], scores, -1000000000.0)
            p = _softmax(scores, axis=-1)
            o = jnp.einsum('bhqk,bhke->bhqe', p, v)
            o = jnp.einsum('bhte,hed->btd', o, Wo)
            mem = o[:, :M, :].copy()
            outs.append(o[:, M:, :])
        return jnp.concatenate(outs, axis=1)
    a = _A_ref(A_x, A_wqkv, A_wo)
    b = _B_ref(B_x, B_mem0, B_Wq, B_Wk, B_Wv, B_Wo, B_seg_len)
    return jnp.concatenate([a, b], axis=-1)
```

```python
import functools

import jax
import jax.numpy as jnp
from jax import lax
import jax.experimental.pallas as pl
import jax.experimental.pallas.tpu as pltpu

F32 = jnp.float32
BF16 = jnp.bfloat16
LANES = 128
MASKED = -1000000000.0

A_HEADS = 32
A_WINDOW = 8
A_DILATION = 2
A_HALO = 16
A_ROWS = 256

_NT = (((1,), (1,)), ((), ()))


def _kernel(
    ax_hbm, awqkv_hbm, awo_hbm, bx_hbm, bmem_hbm, wq_hbm, wk_hbm, wv_hbm, wo_hbm,
    out_hbm,
    ax, awqkv, awo, awqkv_p, awo_p, kbuf, vbuf, aout,
    bx, bmem, wt, wqkv, wo, o_buf, bout,
    sem_aw, sem_ax, sem_wt, sem_b, sem_out,
    *, seg, head_dim,
):
    S, D = ax.shape
    M = bmem.shape[0]
    L = M + seg
    n_seg = S // seg
    n_pair, _, pair3 = wqkv.shape
    pair = pair3 // 3
    n_chunk = S // A_ROWS
    pairs_per_chunk = n_pair // n_chunk
    wt_rows = pairs_per_chunk * pair
    n_tile = D // LANES
    a_dh = D // A_HEADS
    bx_head = 8 * seg

    cp_awqkv = pltpu.make_async_copy(awqkv_hbm, awqkv, sem_aw.at[0])
    cp_awo = pltpu.make_async_copy(awo_hbm, awo, sem_aw.at[1])

    def cp_ax(i):
        rows = pl.ds(pl.multiple_of(i * A_ROWS, A_ROWS), A_ROWS)
        return pltpu.make_async_copy(ax_hbm.at[rows], ax.at[rows], sem_ax.at[i])

    def cp_wt(i):
        rows = pl.ds(pl.multiple_of(i * wt_rows, wt_rows), wt_rows)
        return [
            pltpu.make_async_copy(w.at[rows], wt.at[n, rows], sem_wt.at[3 * i + n])
            for n, w in enumerate((wq_hbm, wk_hbm, wv_hbm))
        ]

    cp_bmem = pltpu.make_async_copy(bmem_hbm, bmem, sem_b.at[0])
    cp_bx0 = pltpu.make_async_copy(
        bx_hbm.at[pl.ds(0, bx_head)], bx.at[pl.ds(0, bx_head)], sem_b.at[1])
    cp_wo = pltpu.make_async_copy(wo_hbm, wo, sem_b.at[2])
    cp_bx1 = pltpu.make_async_copy(
        bx_hbm.at[pl.ds(bx_head, S - bx_head)],
        bx.at[pl.ds(bx_head, S - bx_head)], sem_b.at[3])
    cp_aout = pltpu.make_async_copy(aout, out_hbm.at[:, pl.ds(0, D)], sem_out.at[0])

    def cp_bout(s):
        rows = pl.ds(pl.multiple_of(s * seg, seg), seg)
        return pltpu.make_async_copy(
            bout.at[rows], out_hbm.at[rows, pl.ds(D, D)], sem_out.at[1])

    cp_awqkv.start()
    cp_awo.start()
    for i in range(n_chunk):
        cp_ax(i).start()
        for c in cp_wt(i):
            c.start()
    cp_bmem.start()
    cp_bx0.start()
    cp_wo.start()
    cp_bx1.start()

    r = lax.broadcasted_iota(jnp.int32, (D, D), 0)
    c = lax.broadcasted_iota(jnp.int32, (D, D), 1)
    shift = A_HEADS.bit_length() - 1
    perm = (r == (c & (A_HEADS - 1)) * a_dh + (c >> shift)).astype(F32).astype(BF16)
    perm_t = (c == (r & (A_HEADS - 1)) * a_dh + (r >> shift)).astype(F32).astype(BF16)
    cp_awqkv.wait()
    for n in range(3):
        cols = slice(n * D, (n + 1) * D)
        awqkv_p[:, cols] = jnp.dot(
            awqkv[:, cols], perm, preferred_element_type=F32).astype(BF16)
    cp_awo.wait()
    awo_p[...] = jnp.dot(perm_t, awo[...], preferred_element_type=F32).astype(BF16)

    a_scale = a_dh ** -0.5

    cp_ax(0).wait()
    kv0 = jnp.dot(ax[0:A_HALO, :], awqkv_p[:, D:3 * D], preferred_element_type=F32)
    for t in range(n_tile):
        kbuf[t, A_ROWS:A_ROWS + A_HALO, :] = jnp.broadcast_to(
            kv0[0:1, t * LANES:(t + 1) * LANES], (A_HALO, LANES))
        vbuf[t, A_ROWS:A_ROWS + A_HALO, :] = jnp.broadcast_to(
            kv0[0:1, D + t * LANES:D + (t + 1) * LANES], (A_HALO, LANES))

    def a_chunk(i, carry):
        @pl.when(i > 0)
        def _():
            cp_ax(i).wait()

        for cp in cp_wt(i):
            cp.wait()

        r0 = pl.multiple_of(i * A_ROWS, A_ROWS)
        for t in range(n_tile):
            kbuf[t, 0:A_HALO, :] = kbuf[t, A_ROWS:A_ROWS + A_HALO, :]
            vbuf[t, 0:A_HALO, :] = vbuf[t, A_ROWS:A_ROWS + A_HALO, :]
        x = ax[pl.ds(r0, A_ROWS), :]
        k = jnp.dot(x, awqkv_p[:, D:2 * D], preferred_element_type=F32)
        for t in range(n_tile):
            kbuf[t, A_HALO:, :] = k[:, t * LANES:(t + 1) * LANES]
        q = jnp.dot(x, awqkv_p[:, 0:D], preferred_element_type=F32)
        v = jnp.dot(x, awqkv_p[:, 2 * D:3 * D], preferred_element_type=F32)
        for t in range(n_tile):
            vbuf[t, A_HALO:, :] = v[:, t * LANES:(t + 1) * LANES]

        pos = r0 + lax.broadcasted_iota(jnp.int32, (A_ROWS, LANES), 0)
        logits = []
        for w in range(A_WINDOW):
            back = w * A_DILATION
            rows = pl.ds(A_HALO - back, A_ROWS)
            acc = q[:, 0:LANES] * kbuf[0, rows, :]
            for t in range(1, n_tile):
                acc = acc + q[:, t * LANES:(t + 1) * LANES] * kbuf[t, rows, :]
            rot = LANES // 2
            while rot >= A_HEADS:
                acc = acc + pltpu.roll(acc, rot, 1)
                rot //= 2
            acc = acc * a_scale
            logits.append(jnp.where(pos >= back, acc, MASKED) if back else acc)
        top = functools.reduce(jnp.maximum, logits)
        e = [jnp.exp(z - top) for z in logits]
        inv = 1.0 / functools.reduce(jnp.add, e)
        o = []
        for t in range(n_tile):
            acc = e[0] * vbuf[t, pl.ds(A_HALO, A_ROWS), :]
            for w in range(1, A_WINDOW):
                acc = acc + e[w] * vbuf[t, pl.ds(A_HALO - w * A_DILATION, A_ROWS), :]
            o.append((acc * inv).astype(BF16))
        aout[pl.ds(r0, A_ROWS), :] = jnp.dot(
            jnp.concatenate(o, axis=1), awo_p[...],
            preferred_element_type=F32).astype(BF16)

        for jj in range(pairs_per_chunk):
            j = i * pairs_per_chunk + jj
            rows = pl.ds(pl.multiple_of(j * pair, pair), pair)
            for n in range(3):
                wqkv[j, :, n * pair:(n + 1) * pair] = wt[n, rows, :].T
        return carry

    lax.fori_loop(0, n_chunk, a_chunk, 0)

    cp_bmem.wait()
    cp_bx0.wait()
    cp_wo.wait()
    cp_aout.start()

    b_scale = head_dim ** -0.5
    row = lax.broadcasted_iota(jnp.int32, (L, 2 * L), 0)
    col = lax.broadcasted_iota(jnp.int32, (L, 2 * L), 1)
    first = col < L
    visible = (row < M) | (row >= jnp.where(first, col, col - L))
    low = lax.broadcasted_iota(jnp.int32, (L, LANES), 1) < head_dim - LANES

    def split_pair(a):
        a0, a1, a2 = (a[:, n * LANES:(n + 1) * LANES] for n in range(3))
        zero = jnp.zeros_like(a0)
        return jnp.concatenate([
            jnp.concatenate([a0, jnp.where(low, a1, 0.0), zero], axis=1),
            jnp.concatenate([zero, jnp.where(low, 0.0, a1), a2], axis=1),
        ], axis=0)

    def b_step(s, mem):
        @pl.when(s == bx_head // seg)
        def _():
            cp_bx1.wait()

        r0 = pl.multiple_of(s * seg, seg)
        h = jnp.concatenate([mem, bx[pl.ds(r0, seg), :].astype(F32)], axis=0)
        qkv, probs = {}, {}
        for t in range(n_pair + 2):
            if t < n_pair:
                qkv[t] = jnp.dot(h, wqkv[t], preferred_element_type=F32)
            if 1 <= t <= n_pair:
                j = t - 1
                sc = lax.dot_general(
                    qkv[j][:, 0:pair], split_pair(qkv[j][:, pair:2 * pair]), _NT,
                    preferred_element_type=F32)
                sc = jnp.where(visible, sc * b_scale, MASKED)
                m0 = jnp.max(jnp.where(first, sc, -jnp.inf), axis=1, keepdims=True)
                m1 = jnp.max(jnp.where(first, -jnp.inf, sc), axis=1, keepdims=True)
                e = jnp.exp(sc - jnp.where(first, m0, m1))
                l0 = jnp.sum(jnp.where(first, e, 0.0), axis=1, keepdims=True)
                l1 = jnp.sum(jnp.where(first, 0.0, e), axis=1, keepdims=True)
                probs[j] = e / jnp.where(first, l0, l1)
            if t >= 2:
                j = t - 2
                o_buf[:, j * pair:(j + 1) * pair] = jnp.dot(
                    probs[j], split_pair(qkv[j][:, 2 * pair:3 * pair]),
                    preferred_element_type=F32)
        res = jnp.dot(o_buf[...], wo[...], preferred_element_type=F32)
        bout[pl.ds(r0, seg), :] = res[M:].astype(BF16)
        cp_bout(s).start()
        return res[:M]

    lax.fori_loop(0, n_seg, b_step, bmem[...].astype(F32))

    cp_aout.wait()
    pltpu.make_async_copy(bout, out_hbm.at[:, pl.ds(D, D)], sem_out.at[1]).wait()


@functools.partial(jax.jit, static_argnames=("B_seg_len",))
def pallas_concat_heads__sliding_local_dilated__memory_aug_recurrent_mem_tr__prompt_kernel(
    A_x: jax.Array,
    A_wqkv: jax.Array,
    A_wo: jax.Array,
    B_x: jax.Array,
    B_mem0: jax.Array,
    B_Wq: jax.Array,
    B_Wk: jax.Array,
    B_Wv: jax.Array,
    B_Wo: jax.Array,
    B_seg_len: int,
):
    B, S, D = A_x.shape
    _, H, Dh = B_Wq.shape
    M = B_mem0.shape[1]
    seg = int(B_seg_len)
    E = H * Dh
    n_pair = H // 2
    n_chunk = S // A_ROWS
    assert B == 1 and B_x.shape == (B, S, D) and D % LANES == 0
    assert 2 * Dh == 3 * LANES and 2 * (M + seg) <= LANES
    assert M % 8 == 0 and seg % 16 == 0 and S % seg == 0 and S > 8 * seg
    assert S % A_ROWS == 0 and n_pair % n_chunk == 0 and H % 2 == 0

    def features_first(w):
        return jnp.transpose(w, (1, 2, 0)).reshape(E, D)

    n_tile = D // LANES
    out = pl.pallas_call(
        functools.partial(_kernel, seg=seg, head_dim=Dh),
        out_shape=jax.ShapeDtypeStruct((S, 2 * D), BF16),
        in_specs=[pl.BlockSpec(memory_space=pl.ANY)] * 9,
        out_specs=pl.BlockSpec(memory_space=pl.ANY),
        scratch_shapes=[
            pltpu.VMEM((S, D), BF16),
            pltpu.VMEM((D, 3 * D), BF16),
            pltpu.VMEM((D, D), BF16),
            pltpu.VMEM((D, 3 * D), BF16),
            pltpu.VMEM((D, D), BF16),
            pltpu.VMEM((n_tile, A_HALO + A_ROWS, LANES), F32),
            pltpu.VMEM((n_tile, A_HALO + A_ROWS, LANES), F32),
            pltpu.VMEM((S, D), BF16),
            pltpu.VMEM((S, D), BF16),
            pltpu.VMEM((M, D), BF16),
            pltpu.VMEM((3, E, D), BF16),
            pltpu.VMEM((n_pair, D, 6 * Dh), BF16),
            pltpu.VMEM((E, D), BF16),
            pltpu.VMEM((M + seg, E), F32),
            pltpu.VMEM((S, D), BF16),
            pltpu.SemaphoreType.DMA((2,)),
            pltpu.SemaphoreType.DMA((n_chunk,)),
            pltpu.SemaphoreType.DMA((3 * n_chunk,)),
            pltpu.SemaphoreType.DMA((4,)),
            pltpu.SemaphoreType.DMA((2,)),
        ],
        compiler_params=pltpu.CompilerParams(vmem_limit_bytes=110 * 1024 * 1024),
        name="local_and_recurrent_attention",
    )(
        A_x.reshape(S, D), A_wqkv, A_wo,
        B_x.reshape(S, D), B_mem0.reshape(M, D),
        features_first(B_Wq), features_first(B_Wk), features_first(B_Wv),
        B_Wo.reshape(E, D),
    )
    return out.reshape(B, S, 2 * D)
```

```python
import functools

import jax
import jax.numpy as jnp
from jax import lax
import jax.experimental.pallas as pl
import jax.experimental.pallas.tpu as pltpu

F32 = jnp.float32
BF16 = jnp.bfloat16
LANES = 128
MASKED = -1000000000.0
LOG2_E = 1.4426950408889634

A_HEADS = 32
A_WINDOW = 8
A_DILATION = 2
A_HALO = 16
A_ROWS = 256
B_UNROLL = 2
B_LAG = 2

_NT = (((1,), (1,)), ((), ()))


def _kernel(
    ax_hbm, awqkv_hbm, awo_hbm, bx_hbm, bmem_hbm, wq_hbm, wk_hbm, wv_hbm, wo_hbm,
    out_hbm,
    ax, awqkv, awo, awqkv_p, awo_p, kbuf, vbuf, aout,
    bx, bmem, wt, wqkv, wo, bout,
    sem_aw, sem_ax, sem_wt, sem_b, sem_out,
    *, seg, head_dim,
):
    S, D = ax.shape
    M = bmem.shape[0]
    L = M + seg
    n_pair, _, pair3 = wqkv.shape
    pair = pair3 // 3
    n_chunk = S // A_ROWS
    pairs_per_chunk = n_pair // n_chunk
    wt_rows = pairs_per_chunk * pair
    n_tile = D // LANES
    a_dh = D // A_HEADS

    cp_awqkv = pltpu.make_async_copy(awqkv_hbm, awqkv, sem_aw.at[0])
    cp_awo = pltpu.make_async_copy(awo_hbm, awo, sem_aw.at[1])

    def cp_ax(i):
        rows = pl.ds(pl.multiple_of(i * A_ROWS, A_ROWS), A_ROWS)
        return pltpu.make_async_copy(ax_hbm.at[rows], ax.at[rows], sem_ax.at[i])

    def cp_wt(i):
        feats = pl.ds(pl.multiple_of(i * wt_rows, wt_rows), wt_rows)
        return [
            pltpu.make_async_copy(w.at[feats], wt.at[n, feats], sem_wt.at[3 * i + n])
            for n, w in enumerate((wq_hbm, wk_hbm, wv_hbm))
        ]

    trip_rows = B_UNROLL * seg
    cp_bmem = pltpu.make_async_copy(bmem_hbm, bmem, sem_b.at[0])
    cp_bx0 = pltpu.make_async_copy(
        bx_hbm.at[pl.ds(0, trip_rows)], bx.at[pl.ds(0, trip_rows)], sem_b.at[1])
    cp_wo = pltpu.make_async_copy(wo_hbm, wo, sem_b.at[2])
    cp_bx1 = pltpu.make_async_copy(
        bx_hbm.at[pl.ds(trip_rows, S - trip_rows)],
        bx.at[pl.ds(trip_rows, S - trip_rows)], sem_b.at[3])
    cp_aout = pltpu.make_async_copy(aout, out_hbm.at[:, pl.ds(0, D)], sem_out.at[0])

    cp_awqkv.start()
    cp_awo.start()

    def issue(i, carry):
        cp_ax(i).start()
        for cp in cp_wt(i):
            cp.start()
        return carry

    lax.fori_loop(0, n_chunk, issue, 0)
    cp_bmem.start()
    cp_bx0.start()
    cp_wo.start()

    down = lax.broadcasted_iota(jnp.int32, (LANES, LANES), 0)
    across = lax.broadcasted_iota(jnp.int32, (LANES, LANES), 1)
    shift = A_HEADS.bit_length() - 1

    def source_lane(lane, tile):
        feature = (lane & (A_HEADS - 1)) * a_dh + (lane >> shift) * n_tile + tile
        return feature & (LANES - 1)

    def pick(tiles, residue, tile):
        out = tiles[0]
        for t in range(1, n_tile):
            out = jnp.where(residue == (tile - t * LANES) % n_tile, tiles[t], out)
        return out

    cp_awqkv.wait()
    lane_residue = lax.broadcasted_iota(jnp.int32, (D // 2, LANES), 1) % n_tile
    for n in range(3):
        tiles = [
            pltpu.bitcast(awqkv[:, pl.ds(n * D + t * LANES, LANES)], jnp.int32)
            for t in range(n_tile)
        ]
        for t in range(n_tile):
            awqkv_p[:, pl.ds(n * D + t * LANES, LANES)] = jnp.dot(
                pltpu.bitcast(pick(tiles, lane_residue, t), BF16),
                (down == source_lane(across, t)).astype(F32).astype(BF16),
                preferred_element_type=F32).astype(BF16)
    cp_awo.wait()
    row_residue = lax.broadcasted_iota(jnp.int32, (LANES, D), 0) % n_tile
    tiles = [awo[pl.ds(t * LANES, LANES), :].astype(F32) for t in range(n_tile)]
    for t in range(n_tile):
        awo_p[pl.ds(t * LANES, LANES), :] = jnp.dot(
            (across == source_lane(down, t)).astype(F32).astype(BF16),
            pick(tiles, row_residue, t).astype(BF16),
            preferred_element_type=F32).astype(BF16)

    a_scale = a_dh ** -0.5

    cp_ax(0).wait()
    kv0 = jnp.dot(ax[0:A_HALO, :], awqkv_p[:, D:3 * D], preferred_element_type=F32)
    for t in range(n_tile):
        kbuf[t, A_ROWS:A_ROWS + A_HALO, :] = jnp.broadcast_to(
            kv0[0:1, t * LANES:(t + 1) * LANES], (A_HALO, LANES))
        vbuf[t, A_ROWS:A_ROWS + A_HALO, :] = jnp.broadcast_to(
            kv0[0:1, D + t * LANES:D + (t + 1) * LANES], (A_HALO, LANES))

    def a_chunk(i, carry):
        @pl.when(i > 0)
        def _():
            cp_ax(i).wait()

        for cp in cp_wt(i):
            cp.wait()

        r0 = pl.multiple_of(i * A_ROWS, A_ROWS)
        for t in range(n_tile):
            kbuf[t, 0:A_HALO, :] = kbuf[t, A_ROWS:A_ROWS + A_HALO, :]
            vbuf[t, 0:A_HALO, :] = vbuf[t, A_ROWS:A_ROWS + A_HALO, :]
        x = ax[pl.ds(r0, A_ROWS), :]
        k = jnp.dot(x, awqkv_p[:, D:2 * D], preferred_element_type=F32)
        for t in range(n_tile):
            kbuf[t, A_HALO:, :] = k[:, t * LANES:(t + 1) * LANES]
        q = jnp.dot(x, awqkv_p[:, 0:D], preferred_element_type=F32)
        v = jnp.dot(x, awqkv_p[:, 2 * D:3 * D], preferred_element_type=F32)
        for t in range(n_tile):
            vbuf[t, A_HALO:, :] = v[:, t * LANES:(t + 1) * LANES]

        pos = r0 + lax.broadcasted_iota(jnp.int32, (A_HALO, LANES), 0)
        logits = []
        for w in range(A_WINDOW):
            back = w * A_DILATION
            rows = pl.ds(A_HALO - back, A_ROWS)
            acc = q[:, 0:LANES] * kbuf[0, rows, :]
            for t in range(1, n_tile):
                acc = acc + q[:, t * LANES:(t + 1) * LANES] * kbuf[t, rows, :]
            rot = LANES // 2
            while rot >= A_HEADS:
                acc = acc + pltpu.roll(acc, rot, 1)
                rot //= 2
            if back:
                head = jnp.where(pos >= back, acc[:A_HALO], MASKED / a_scale)
                acc = jnp.concatenate([head, acc[A_HALO:]], axis=0)
            logits.append(acc)
        top = functools.reduce(jnp.maximum, logits)
        e = [jnp.exp2((z - top) * (a_scale * LOG2_E)) for z in logits]
        inv = 1.0 / functools.reduce(jnp.add, e)
        o = []
        for t in range(n_tile):
            acc = e[0] * vbuf[t, pl.ds(A_HALO, A_ROWS), :]
            for w in range(1, A_WINDOW):
                acc = acc + e[w] * vbuf[t, pl.ds(A_HALO - w * A_DILATION, A_ROWS), :]
            o.append((acc * inv).astype(BF16))
        aout[pl.ds(r0, A_ROWS), :] = jnp.dot(
            jnp.concatenate(o, axis=1), awo_p[...],
            preferred_element_type=F32).astype(BF16)

        for jj in range(pairs_per_chunk):
            j = i * pairs_per_chunk + jj
            feats = pl.ds(pl.multiple_of(j * pair, pair), pair)
            for n in range(3):
                wqkv[j, :, n * pair:(n + 1) * pair] = wt[n, feats, :].T
        return carry

    lax.fori_loop(0, n_chunk, a_chunk, 0)

    cp_bx1.start()
    cp_bmem.wait()
    cp_bx0.wait()
    cp_wo.wait()

    b_scale = head_dim ** -0.5
    row = lax.broadcasted_iota(jnp.int32, (L, 2 * L), 0)
    col = lax.broadcasted_iota(jnp.int32, (L, 2 * L), 1)
    first = col < L
    visible = (row < M) | (row >= jnp.where(first, col, col - L))
    low = lax.broadcasted_iota(jnp.int32, (L, LANES), 1) < head_dim - LANES

    def split_pair(a):
        a0, a1, a2 = (a[:, n * LANES:(n + 1) * LANES] for n in range(3))
        zero = jnp.zeros_like(a0)
        return jnp.concatenate([
            jnp.concatenate([a0, jnp.where(low, a1, 0.0), zero], axis=1),
            jnp.concatenate([zero, jnp.where(low, 0.0, a1), a2], axis=1),
        ], axis=0)

    def attention_weights(qkv):
        sc = lax.dot_general(
            qkv[:, 0:pair], split_pair(qkv[:, pair:2 * pair]), _NT,
            preferred_element_type=F32)
        sc = jnp.where(visible, sc * b_scale, MASKED)
        m0 = jnp.max(jnp.where(first, sc, -jnp.inf), axis=1, keepdims=True)
        m1 = jnp.max(jnp.where(first, -jnp.inf, sc), axis=1, keepdims=True)
        e = jnp.exp(sc - jnp.where(first, m0, m1))
        l0 = jnp.sum(jnp.where(first, e, 0.0), axis=1, keepdims=True)
        l1 = jnp.sum(jnp.where(first, 0.0, e), axis=1, keepdims=True)
        return e / jnp.where(first, l0, l1)

    def segment(r0, mem):
        h = jnp.concatenate([mem, bx[pl.ds(r0, seg), :].astype(F32)], axis=0)
        qkv, probs, o = {}, {}, {}
        res, done = None, 0
        for t in range(n_pair + 2 * B_LAG + 1):
            if t < n_pair:
                qkv[t] = jnp.dot(h, wqkv[t], preferred_element_type=F32)
            else:
                upto = n_pair * (t - n_pair + 1) // (2 * B_LAG + 1)
                part = jnp.dot(
                    jnp.concatenate([o[j] for j in range(done, upto)], axis=1),
                    wo[done * pair:upto * pair, :], preferred_element_type=F32)
                res = part if res is None else res + part
                done = upto
            j = t - B_LAG
            if 0 <= j < n_pair:
                probs[j] = attention_weights(qkv[j])
            j = t - 2 * B_LAG
            if 0 <= j < n_pair:
                o[j] = jnp.dot(
                    probs[j], split_pair(qkv[j][:, 2 * pair:3 * pair]),
                    preferred_element_type=F32)
        bout[pl.ds(r0, seg), :] = res[M:].astype(BF16)
        return res[:M]

    def b_trip(i, mem):
        @pl.when(i == 1)
        def _():
            cp_bx1.wait()
            cp_aout.start()

        for u in range(B_UNROLL):
            mem = segment(pl.multiple_of(i * trip_rows + u * seg, seg), mem)
        rows = pl.ds(pl.multiple_of(i * trip_rows, trip_rows), trip_rows)
        pltpu.make_async_copy(
            bout.at[rows], out_hbm.at[rows, pl.ds(D, D)], sem_out.at[1]).start()
        return mem

    lax.fori_loop(0, S // trip_rows, b_trip, bmem[...].astype(F32))

    cp_aout.wait()
    pltpu.make_async_copy(bout, out_hbm.at[:, pl.ds(D, D)], sem_out.at[1]).wait()


@functools.partial(jax.jit, static_argnames=("B_seg_len",))
def pallas_concat_heads__sliding_local_dilated__memory_aug_recurrent_mem_tr__prompt_kernel(
    A_x: jax.Array,
    A_wqkv: jax.Array,
    A_wo: jax.Array,
    B_x: jax.Array,
    B_mem0: jax.Array,
    B_Wq: jax.Array,
    B_Wk: jax.Array,
    B_Wv: jax.Array,
    B_Wo: jax.Array,
    B_seg_len: int,
):
    B, S, D = A_x.shape
    _, H, Dh = B_Wq.shape
    M = B_mem0.shape[1]
    seg = int(B_seg_len)
    E = H * Dh
    n_pair = H // 2
    n_chunk = S // A_ROWS
    assert B == 1 and B_x.shape == (B, S, D) and D % LANES == 0
    assert 2 * Dh == 3 * LANES and 2 * (M + seg) <= LANES
    assert M % 8 == 0 and seg % 16 == 0
    assert S % (B_UNROLL * seg) == 0 and S >= 2 * B_UNROLL * seg
    assert (D // LANES) % 2 == 1
    assert S % A_ROWS == 0 and n_pair % n_chunk == 0 and H % 2 == 0

    def features_first(w):
        return jnp.transpose(w, (1, 2, 0)).reshape(E, D)

    n_tile = D // LANES
    out = pl.pallas_call(
        functools.partial(_kernel, seg=seg, head_dim=Dh),
        out_shape=jax.ShapeDtypeStruct((S, 2 * D), BF16),
        in_specs=[pl.BlockSpec(memory_space=pl.ANY)] * 9,
        out_specs=pl.BlockSpec(memory_space=pl.ANY),
        scratch_shapes=[
            pltpu.VMEM((S, D), BF16),
            pltpu.VMEM((D, 3 * D), BF16),
            pltpu.VMEM((D, D), BF16),
            pltpu.VMEM((D, 3 * D), BF16),
            pltpu.VMEM((D, D), BF16),
            pltpu.VMEM((n_tile, A_HALO + A_ROWS, LANES), F32),
            pltpu.VMEM((n_tile, A_HALO + A_ROWS, LANES), F32),
            pltpu.VMEM((S, D), BF16),
            pltpu.VMEM((S, D), BF16),
            pltpu.VMEM((M, D), BF16),
            pltpu.VMEM((3, E, D), BF16),
            pltpu.VMEM((n_pair, D, 6 * Dh), BF16),
            pltpu.VMEM((E, D), BF16),
            pltpu.VMEM((S, D), BF16),
            pltpu.SemaphoreType.DMA((2,)),
            pltpu.SemaphoreType.DMA((n_chunk,)),
            pltpu.SemaphoreType.DMA((3 * n_chunk,)),
            pltpu.SemaphoreType.DMA((4,)),
            pltpu.SemaphoreType.DMA((2,)),
        ],
        compiler_params=pltpu.CompilerParams(vmem_limit_bytes=110 * 1024 * 1024),
        name="local_and_recurrent_attention",
    )(
        A_x.reshape(S, D), A_wqkv, A_wo,
        B_x.reshape(S, D), B_mem0.reshape(M, D),
        features_first(B_Wq), features_first(B_Wk), features_first(B_Wv),
        B_Wo.reshape(E, D),
    )
    return out.reshape(B, S, 2 * D)
```

```python
import functools

import jax
import jax.numpy as jnp
from jax import lax
import jax.experimental.pallas as pl
import jax.experimental.pallas.tpu as pltpu

F32 = jnp.float32
BF16 = jnp.bfloat16
LANES = 128
MASKED = -1000000000.0
LOG2_E = 1.4426950408889634

A_HEADS = 32
A_WINDOW = 8
A_DILATION = 2
A_HALO = 16
A_ROWS = 256
A_BLOCK = 64
A_GROUP = 16
B_UNROLL = 3
B_LAG = 2

_NT = (((1,), (1,)), ((), ()))


def _pack(w):
    return pltpu.bitcast(w, jnp.int32)


def _unpack(w):
    return pltpu.bitcast(w, BF16)


def _dot(a, b):
    return jnp.dot(a, b, preferred_element_type=F32)


def _kernel(
    ax_hbm, awqkv_hbm, awo_hbm, bx_hbm, bmem_hbm, wq_hbm, wk_hbm, wv_hbm, wo_hbm,
    out_hbm,
    ax, awqkv, awo, awqkv_p, awo_p, kbuf, vbuf, aout,
    bx, bmem, wt, wqkv, wo, bout,
    sem_aw, sem_ax, sem_wt, sem_wo, sem_b, sem_out,
    *, seg, head_dim,
):
    S, D = ax.shape
    M = bmem.shape[0]
    L = M + seg
    n_pair = wqkv.shape[0]
    pair = 2 * head_dim
    n_trip = S // A_ROWS
    pairs_per_trip = n_pair // n_trip
    n_tile = D // LANES
    a_dh = D // A_HEADS
    trip_rows = B_UNROLL * seg
    early_rows = seg + trip_rows

    cp_awqkv = pltpu.make_async_copy(awqkv_hbm, awqkv, sem_aw.at[0])
    cp_awo = pltpu.make_async_copy(awo_hbm, awo, sem_aw.at[1])

    def cp_ax(i):
        rows = pl.ds(pl.multiple_of(i * A_ROWS, A_ROWS), A_ROWS)
        return pltpu.make_async_copy(ax_hbm.at[rows], ax.at[rows], sem_ax.at[i])

    def cp_wt(j):
        feats = pl.ds(pl.multiple_of(j * pair, pair), pair)
        return [
            pltpu.make_async_copy(w.at[feats], wt.at[n, feats], sem_wt.at[3 * j + n])
            for n, w in enumerate((wq_hbm, wk_hbm, wv_hbm))
        ]

    def cp_wo(j):
        feats = pl.ds(pl.multiple_of(j * pair, pair), pair)
        return pltpu.make_async_copy(wo_hbm.at[feats], wo.at[feats], sem_wo.at[j])

    cp_bmem = pltpu.make_async_copy(bmem_hbm, bmem, sem_b.at[0])
    cp_bx_early = pltpu.make_async_copy(
        bx_hbm.at[pl.ds(0, early_rows)], bx.at[pl.ds(0, early_rows)], sem_b.at[1])
    cp_bx_rest = pltpu.make_async_copy(
        bx_hbm.at[pl.ds(early_rows, S - early_rows)],
        bx.at[pl.ds(early_rows, S - early_rows)], sem_b.at[2])
    cp_aout = pltpu.make_async_copy(aout, out_hbm.at[:, pl.ds(0, D)], sem_out.at[0])

    def cp_bout(r0, n):
        rows = pl.ds(r0, n)
        return pltpu.make_async_copy(
            bout.at[rows], out_hbm.at[rows, pl.ds(D, D)], sem_out.at[1])

    late_pairs = range(n_pair - pairs_per_trip + 1, n_pair)

    def trip_inputs(i, action):
        action(cp_ax(i))
        for back in range(pairs_per_trip - 1, 0, -1):
            @pl.when(i > 0)
            def _(back=back):
                for cp in cp_wt(i * pairs_per_trip - back):
                    action(cp)

        for cp in cp_wt(i * pairs_per_trip):
            action(cp)

    def transpose_weights(j, n):
        feats = pl.ds(pl.multiple_of(j * pair, pair), pair)
        wqkv[j, :, n * pair:(n + 1) * pair] = _pack(wt[n, feats, :].T)

    cp_awqkv.start()
    cp_awo.start()

    @pl.loop(0, n_trip)
    def _(i):
        trip_inputs(i, lambda cp: cp.start())

    for j in late_pairs:
        for cp in cp_wt(j):
            cp.start()
    cp_bmem.start()
    cp_bx_early.start()

    @pl.loop(0, n_pair)
    def _(j):
        cp_wo(j).start()

    down = lax.broadcasted_iota(jnp.int32, (LANES, LANES), 0)
    across = lax.broadcasted_iota(jnp.int32, (LANES, LANES), 1)
    shift = A_HEADS.bit_length() - 1

    def source_lane(lane, tile):
        feature = (lane & (A_HEADS - 1)) * a_dh + (lane >> shift) * n_tile + tile
        return feature & (LANES - 1)

    def pick(tiles, residue, tile):
        out = tiles[0]
        for t in range(1, n_tile):
            out = jnp.where(residue == (tile - t * LANES) % n_tile, tiles[t], out)
        return out

    cp_awqkv.wait()

    @pl.loop(0, 3)
    def _(n):
        def lanes(t):
            return pl.ds(pl.multiple_of(n * D + t * LANES, LANES), LANES)

        residue = lax.broadcasted_iota(jnp.int32, (D // 2, LANES), 1) % n_tile
        tiles = [_pack(awqkv[:, lanes(t)]) for t in range(n_tile)]
        for t in range(n_tile):
            awqkv_p[n, :, t * LANES:(t + 1) * LANES] = _pack(_dot(
                _unpack(pick(tiles, residue, t)),
                (down == source_lane(across, t)).astype(F32).astype(BF16),
            ).astype(BF16))

    cp_awo.wait()
    residue = lax.broadcasted_iota(jnp.int32, (LANES, D), 0) % n_tile
    tiles = [awo[pl.ds(t * LANES, LANES), :].astype(F32) for t in range(n_tile)]
    for t in range(n_tile):
        awo_p[pl.ds(t * LANES // 2, LANES // 2), :] = _pack(_dot(
            (across == source_lane(down, t)).astype(F32).astype(BF16),
            pick(tiles, residue, t).astype(BF16),
        ).astype(BF16))

    a_scale = a_dh ** -0.5

    def a_rows(i, block):
        return pl.ds(pl.multiple_of(i * A_ROWS + block * A_BLOCK, A_BLOCK), A_BLOCK)

    def a_project(i, block):
        x = ax[a_rows(i, block), :]
        k = _dot(x, _unpack(awqkv_p[1]))
        q = _dot(x, _unpack(awqkv_p[0]))
        v = _dot(x, _unpack(awqkv_p[2]))
        for buf, val in ((kbuf, k), (vbuf, v)):
            for t in range(n_tile):
                buf[t, pl.ds(A_HALO + block * A_BLOCK, A_BLOCK), :] = (
                    val[:, t * LANES:(t + 1) * LANES])
        return q

    def a_attend(i, block, q_block):
        out = []
        for g0 in range(0, A_BLOCK, A_GROUP):
            q = q_block[g0:g0 + A_GROUP]
            at = block * A_BLOCK + g0

            def window(buf, t, w):
                return buf[t, pl.ds(A_HALO + at - w * A_DILATION, A_GROUP), :]

            logits = []
            for w in range(A_WINDOW):
                z = functools.reduce(jnp.add, [
                    q[:, t * LANES:(t + 1) * LANES] * window(kbuf, t, w)
                    for t in range(n_tile)])
                rot = LANES // 2
                while rot >= A_HEADS:
                    z = z + pltpu.roll(z, rot, 1)
                    rot //= 2
                if w * A_DILATION > at:
                    pos = i * A_ROWS + at + lax.broadcasted_iota(jnp.int32, z.shape, 0)
                    z = jnp.where(pos >= w * A_DILATION, z, MASKED / a_scale)
                logits.append(z)
            top = functools.reduce(jnp.maximum, logits)
            e = [jnp.exp2((z - top) * (a_scale * LOG2_E)) for z in logits]
            inv = 1.0 / functools.reduce(jnp.add, e)
            out.append(jnp.concatenate([
                functools.reduce(
                    jnp.add, [e[w] * window(vbuf, t, w) for w in range(A_WINDOW)]) * inv
                for t in range(n_tile)], axis=1))
        return jnp.concatenate(out, axis=0).astype(BF16)

    @pl.loop(0, n_trip)
    def _(i):
        trip_inputs(i, lambda cp: cp.wait())

        @pl.when(i == 0)
        def _():
            for buf, n in ((kbuf, 1), (vbuf, 2)):
                row0 = _dot(ax[0:A_HALO, :], _unpack(awqkv_p[n]))[0:1]
                for t in range(n_tile):
                    buf[t, A_ROWS:, :] = jnp.broadcast_to(
                        row0[:, t * LANES:(t + 1) * LANES], (A_HALO, LANES))

        for buf in (kbuf, vbuf):
            for t in range(n_tile):
                buf[t, 0:A_HALO, :] = buf[t, A_ROWS:, :]

        turns = [
            (jnp.maximum(i * pairs_per_trip - back, 0), n)
            for back in range(pairs_per_trip - 1, -1, -1) for n in range(3)]
        n_block = A_ROWS // A_BLOCK
        q, o = {}, {}
        for t in range(2 * n_block):
            if t < n_block:
                q[t] = a_project(i, t)
            else:
                aout[a_rows(i, t - n_block), :] = _dot(
                    o[t - n_block], _unpack(awo_p[...])).astype(BF16)
            if 1 <= t <= n_block:
                o[t - 1] = a_attend(i, t - 1, q[t - 1])
            if turns and t != n_block - 1:
                transpose_weights(*turns.pop(0))
        for turn in turns:
            transpose_weights(*turn)

    b_scale = head_dim ** -0.5
    row = lax.broadcasted_iota(jnp.int32, (L, 2 * L), 0)
    col = lax.broadcasted_iota(jnp.int32, (L, 2 * L), 1)
    first = col < L
    visible = (row < M) | (row >= jnp.where(first, col, col - L))
    low = lax.broadcasted_iota(jnp.int32, (L, LANES), 1) < head_dim - LANES

    def split_pair(a):
        a0, a1, a2 = (a[:, n * LANES:(n + 1) * LANES] for n in range(3))
        zero = jnp.zeros_like(a0)
        return jnp.concatenate([
            jnp.concatenate([a0, jnp.where(low, a1, 0.0), zero], axis=1),
            jnp.concatenate([zero, jnp.where(low, 0.0, a1), a2], axis=1),
        ], axis=0)

    def attention_weights(qkv):
        sc = lax.dot_general(
            qkv[:, 0:pair], split_pair(qkv[:, pair:2 * pair]), _NT,
            preferred_element_type=F32)
        sc = jnp.where(visible, sc * b_scale, MASKED)
        m0 = jnp.max(jnp.where(first, sc, -jnp.inf), axis=1, keepdims=True)
        m1 = jnp.max(jnp.where(first, -jnp.inf, sc), axis=1, keepdims=True)
        e = jnp.exp(sc - jnp.where(first, m0, m1))
        l0 = jnp.sum(jnp.where(first, e, 0.0), axis=1, keepdims=True)
        l1 = jnp.sum(jnp.where(first, 0.0, e), axis=1, keepdims=True)
        return e / jnp.where(first, l0, l1)

    def segment(r0, mem, wo_in_flight=False):
        h = jnp.concatenate([mem, bx[pl.ds(r0, seg), :].astype(F32)], axis=0)
        qkv, probs, o = {}, {}, {}
        res, done = None, 0
        for t in range(n_pair + 2 * B_LAG + 1):
            if t == 0:
                w = _unpack(wqkv[0])
                cut = D - LANES
                q = _dot(h[:, :cut], w[:cut, :pair])
                q = _dot(h[:, cut:], w[cut:, :pair]) + q
                qkv[t] = jnp.concatenate([q, _dot(h, w[:, pair:])], axis=1)
            elif t < n_pair:
                qkv[t] = _dot(h, _unpack(wqkv[t]))
            else:
                upto = n_pair * (t - n_pair + 1) // (2 * B_LAG + 1)
                if wo_in_flight:
                    for j in range(done, upto):
                        cp_wo(j).wait()
                part = _dot(
                    jnp.concatenate([o[j] for j in range(done, upto)], axis=1),
                    wo[done * pair:upto * pair, :])
                res = part if res is None else part + res
                done = upto
            j = t - B_LAG
            if 0 <= j < n_pair:
                probs[j] = attention_weights(qkv[j])
            j = t - 2 * B_LAG
            if 0 <= j < n_pair:
                o[j] = _dot(probs[j], split_pair(qkv[j][:, 2 * pair:3 * pair]))
        bout[pl.ds(r0, seg), :] = res[M:].astype(BF16)
        return res[:M]

    cp_bx_rest.start()
    cp_bmem.wait()
    cp_bx_early.wait()
    for j in late_pairs:
        for cp in cp_wt(j):
            cp.wait()
    for j in late_pairs:
        for n in range(3):
            transpose_weights(j, n)
    mem = segment(0, bmem[...].astype(F32), wo_in_flight=True)
    cp_aout.start()
    cp_bout(0, seg).start()

    def b_trip(i, mem):
        @pl.when(i == 1)
        def _():
            cp_bx_rest.wait()

        r0 = pl.multiple_of(seg + i * trip_rows, seg)
        for u in range(B_UNROLL):
            mem = segment(pl.multiple_of(r0 + u * seg, seg), mem)
        cp_bout(r0, trip_rows).start()
        return mem

    lax.fori_loop(0, (S - seg) // trip_rows, b_trip, mem)

    cp_aout.wait()
    cp_bout(0, S).wait()


@functools.partial(jax.jit, static_argnames=("B_seg_len",))
def pallas_concat_heads__sliding_local_dilated__memory_aug_recurrent_mem_tr__prompt_kernel(
    A_x: jax.Array,
    A_wqkv: jax.Array,
    A_wo: jax.Array,
    B_x: jax.Array,
    B_mem0: jax.Array,
    B_Wq: jax.Array,
    B_Wk: jax.Array,
    B_Wv: jax.Array,
    B_Wo: jax.Array,
    B_seg_len: int,
):
    B, S, D = A_x.shape
    _, H, Dh = B_Wq.shape
    M = B_mem0.shape[1]
    seg = int(B_seg_len)
    E = H * Dh
    n_pair = H // 2
    n_trip = S // A_ROWS
    n_tile = D // LANES
    assert B == 1 and B_x.shape == (B, S, D)
    assert D % LANES == 0 and n_tile % 2 == 1
    assert H % 2 == 0 and 2 * Dh == 3 * LANES and 2 * (M + seg) <= LANES
    assert M % 8 == 0 and seg % 16 == 0 and S % seg == 0
    assert (S // seg - 1) % B_UNROLL == 0 and S // seg > 2 * B_UNROLL
    assert S % A_ROWS == 0 and n_pair % n_trip == 0

    def features_first(w):
        return jnp.transpose(w, (1, 2, 0)).reshape(E, D)

    out = pl.pallas_call(
        functools.partial(_kernel, seg=seg, head_dim=Dh),
        out_shape=jax.ShapeDtypeStruct((S, 2 * D), BF16),
        in_specs=[pl.BlockSpec(memory_space=pl.ANY)] * 9,
        out_specs=pl.BlockSpec(memory_space=pl.ANY),
        scratch_shapes=[
            pltpu.VMEM((S, D), BF16),
            pltpu.VMEM((D, 3 * D), BF16),
            pltpu.VMEM((D, D), BF16),
            pltpu.VMEM((3, D // 2, D), jnp.int32),
            pltpu.VMEM((D // 2, D), jnp.int32),
            pltpu.VMEM((n_tile, A_HALO + A_ROWS, LANES), F32),
            pltpu.VMEM((n_tile, A_HALO + A_ROWS, LANES), F32),
            pltpu.VMEM((S, D), BF16),
            pltpu.VMEM((S, D), BF16),
            pltpu.VMEM((M, D), BF16),
            pltpu.VMEM((3, E, D), BF16),
            pltpu.VMEM((n_pair, D // 2, 6 * Dh), jnp.int32),
            pltpu.VMEM((E, D), BF16),
            pltpu.VMEM((S, D), BF16),
            pltpu.SemaphoreType.DMA((2,)),
            pltpu.SemaphoreType.DMA((n_trip,)),
            pltpu.SemaphoreType.DMA((3 * n_pair,)),
            pltpu.SemaphoreType.DMA((n_pair,)),
            pltpu.SemaphoreType.DMA((3,)),
            pltpu.SemaphoreType.DMA((2,)),
        ],
        compiler_params=pltpu.CompilerParams(vmem_limit_bytes=110 * 1024 * 1024),
        name="local_and_recurrent_attention",
    )(
        A_x.reshape(S, D), A_wqkv, A_wo,
        B_x.reshape(S, D), B_mem0.reshape(M, D),
        features_first(B_Wq), features_first(B_Wk), features_first(B_Wv),
        B_Wo.reshape(E, D),
    )
    return out.reshape(B, S, 2 * D)
```

```python
import functools

import jax
import jax.numpy as jnp
from jax import lax
import jax.experimental.pallas as pl
import jax.experimental.pallas.tpu as pltpu

F32 = jnp.float32
BF16 = jnp.bfloat16
LANES = 128
MASKED = -1000000000.0
LOG2_E = 1.4426950408889634

A_HEADS = 32
A_WINDOW = 8
A_DILATION = 2
A_HALO = 16
A_ROWS = 256
A_BLOCK = 64
A_GROUP = 16
A_TURNS = (0, 1, 2, 4, 5, 6)
B_UNROLL = 3
B_LAG = 2
WO_EARLY_PARTS = 2

_NT = (((1,), (1,)), ((), ()))


def _pack(w):
    return pltpu.bitcast(w, jnp.int32)


def _unpack(w):
    return pltpu.bitcast(w, BF16)


def _dot(a, b):
    return jnp.dot(a, b, preferred_element_type=F32)


def _kernel(
    ax_hbm, awqkv_hbm, awo_hbm, bx_hbm, bmem_hbm, wq_hbm, wk_hbm, wv_hbm, wo_hbm,
    out_hbm,
    ax, awqkv, awo, awqkv_p, awo_p, kbuf, vbuf, aout,
    bx, bmem, wt, wqkv, wo, bout,
    sems,
    *, seg, head_dim,
):
    S, D = ax.shape
    M = bmem.shape[0]
    L = M + seg
    n_slab = wqkv.shape[0]
    n_pair = n_slab // 3
    pair = 2 * head_dim
    n_trip = S // A_ROWS
    n_tile = D // LANES
    a_dh = D // A_HEADS
    trip_rows = B_UNROLL * seg
    early_rows = seg + trip_rows
    n_part = 2 * B_LAG + 1
    early_pairs = n_pair * WO_EARLY_PARTS // n_part

    def rows_of(src, dst, start, size, sem):
        rows = pl.ds(start, size)
        return pltpu.make_async_copy(src.at[rows], dst.at[rows], sems.at[sem])

    def cp_awqkv(n):
        cols = pl.ds(pl.multiple_of(n * D, D), D)
        return pltpu.make_async_copy(awqkv_hbm.at[:, cols], awqkv.at[n], sems.at[n])

    def cp_slab(j, n, sem):
        feats = pl.ds(pl.multiple_of(j * pair, pair), pair)
        return pltpu.make_async_copy(
            (wq_hbm, wk_hbm, wv_hbm)[n].at[feats], wt.at[3 * j + n], sems.at[sem])

    def turn_weights(slab):
        wqkv[slab] = _pack(wt[slab].T)

    trip_slabs = n_slab // n_trip
    late_slabs = range(n_slab - trip_slabs + 1, n_slab)

    def trip_inputs(i, action):
        @pl.when(i > 0)
        def _():
            action(rows_of(
                ax_hbm, ax, pl.multiple_of(i * A_ROWS, A_ROWS), A_ROWS, 9 + i))
            for k in range(1 - trip_slabs, 0):
                action(cp_slab(i * (trip_slabs // 3) + k // 3, k % 3, 9 + i))

        action(cp_slab(i * (trip_slabs // 3), 0, 9 + i))

    cp_awo = pltpu.make_async_copy(awo_hbm, awo, sems.at[3])
    cp_ax_first = rows_of(ax_hbm, ax, 0, A_ROWS, 8)
    cp_b_first = [cp_slab(k // 3, k % 3, 4) for k in late_slabs] + [
        pltpu.make_async_copy(bmem_hbm, bmem, sems.at[4]),
        rows_of(bx_hbm, bx, 0, early_rows, 4),
        rows_of(wo_hbm, wo, 0, early_pairs * pair, 4),
    ]
    cp_wo_rest = rows_of(
        wo_hbm, wo, early_pairs * pair, (n_pair - early_pairs) * pair, 5)
    cp_bx_rest = rows_of(bx_hbm, bx, early_rows, S - early_rows, 6)
    cp_aout = pltpu.make_async_copy(aout, out_hbm.at[:, pl.ds(0, D)], sems.at[7])

    def cp_bout(r0, n):
        rows = pl.ds(r0, n)
        return pltpu.make_async_copy(
            bout.at[rows], out_hbm.at[rows, pl.ds(D, D)], sems.at[7])

    cp_awo.start()

    @pl.loop(0, 3)
    def _(n):
        cp_awqkv(n).start()

    cp_ax_first.start()

    @pl.loop(0, n_trip)
    def _(i):
        trip_inputs(i, lambda cp: cp.start())

    for cp in cp_b_first:
        cp.start()

    down = lax.broadcasted_iota(jnp.int32, (LANES, LANES), 0)
    across = lax.broadcasted_iota(jnp.int32, (LANES, LANES), 1)
    shift = A_HEADS.bit_length() - 1

    def source_lane(lane, tile):
        feature = (lane & (A_HEADS - 1)) * a_dh + (lane >> shift) * n_tile + tile
        return feature & (LANES - 1)

    def pick(tiles, residue, tile):
        out = tiles[0]
        for t in range(1, n_tile):
            out = jnp.where(residue == (tile - t * LANES) % n_tile, tiles[t], out)
        return out

    cp_awo.wait()
    residue = lax.broadcasted_iota(jnp.int32, (LANES, D), 0) % n_tile
    tiles = [awo[pl.ds(t * LANES, LANES), :].astype(F32) for t in range(n_tile)]
    for t in range(n_tile):
        awo_p[pl.ds(t * LANES // 2, LANES // 2), :] = _pack(_dot(
            (across == source_lane(down, t)).astype(F32).astype(BF16),
            pick(tiles, residue, t).astype(BF16),
        ).astype(BF16))

    @pl.loop(0, 3)
    def _(n):
        cp_awqkv(n).wait()
        residue = lax.broadcasted_iota(jnp.int32, (D // 2, LANES), 1) % n_tile
        tiles = [
            _pack(awqkv[n, :, t * LANES:(t + 1) * LANES]) for t in range(n_tile)]
        for t in range(n_tile):
            awqkv_p[n, :, t * LANES:(t + 1) * LANES] = _pack(_dot(
                _unpack(pick(tiles, residue, t)),
                (down == source_lane(across, t)).astype(F32).astype(BF16),
            ).astype(BF16))

    cp_wo_rest.start()
    cp_ax_first.wait()

    for buf, n in ((kbuf, 1), (vbuf, 2)):
        row0 = _dot(ax[0:A_HALO, :], _unpack(awqkv_p[n]))[0:1]
        for t in range(n_tile):
            buf[t, A_ROWS:, :] = jnp.broadcast_to(
                row0[:, t * LANES:(t + 1) * LANES], (A_HALO, LANES))

    a_scale = a_dh ** -0.5

    def a_rows(i, block):
        return pl.ds(pl.multiple_of(i * A_ROWS + block * A_BLOCK, A_BLOCK), A_BLOCK)

    def a_project(i, block):
        x = ax[a_rows(i, block), :]
        k = _dot(x, _unpack(awqkv_p[1]))
        q = _dot(x, _unpack(awqkv_p[0]))
        v = _dot(x, _unpack(awqkv_p[2]))
        for buf, val in ((kbuf, k), (vbuf, v)):
            for t in range(n_tile):
                buf[t, pl.ds(A_HALO + block * A_BLOCK, A_BLOCK), :] = (
                    val[:, t * LANES:(t + 1) * LANES])
        return q

    def a_attend(i, block, q_block):
        out = []
        for g0 in range(0, A_BLOCK, A_GROUP):
            q = q_block[g0:g0 + A_GROUP]
            at = block * A_BLOCK + g0

            def window(buf, t, w):
                return buf[t, pl.ds(A_HALO + at - w * A_DILATION, A_GROUP), :]

            logits = []
            for w in range(A_WINDOW):
                z = functools.reduce(jnp.add, [
                    q[:, t * LANES:(t + 1) * LANES] * window(kbuf, t, w)
                    for t in range(n_tile)])
                rot = LANES // 2
                while rot >= A_HEADS:
                    z = z + pltpu.roll(z, rot, 1)
                    rot //= 2
                if w * A_DILATION > at:
                    pos = i * A_ROWS + at + lax.broadcasted_iota(jnp.int32, z.shape, 0)
                    z = jnp.where(pos >= w * A_DILATION, z, MASKED / a_scale)
                logits.append(z)
            top = functools.reduce(jnp.maximum, logits)
            e = [jnp.exp2((z - top) * (a_scale * LOG2_E)) for z in logits]
            inv = 1.0 / functools.reduce(jnp.add, e)
            out.append(jnp.concatenate([
                functools.reduce(
                    jnp.add, [e[w] * window(vbuf, t, w) for w in range(A_WINDOW)]) * inv
                for t in range(n_tile)], axis=1))
        return jnp.concatenate(out, axis=0).astype(BF16)

    @pl.loop(0, n_trip)
    def _(i):
        trip_inputs(i, lambda cp: cp.wait())
        for buf in (kbuf, vbuf):
            for t in range(n_tile):
                buf[t, 0:A_HALO, :] = buf[t, A_ROWS:, :]

        n_block = A_ROWS // A_BLOCK
        q, o = {}, {}
        for t in range(2 * n_block):
            if t < n_block:
                q[t] = a_project(i, t)
            else:
                aout[a_rows(i, t - n_block), :] = _dot(
                    o[t - n_block], _unpack(awo_p[...])).astype(BF16)
            if 1 <= t <= n_block:
                o[t - 1] = a_attend(i, t - 1, q[t - 1])
            for k in range(trip_slabs):
                if A_TURNS[k % len(A_TURNS)] == t:
                    turn_weights(
                        jnp.maximum(i * trip_slabs + k + 1 - trip_slabs, 0))

    b_scale = head_dim ** -0.5
    row = lax.broadcasted_iota(jnp.int32, (L, 2 * L), 0)
    col = lax.broadcasted_iota(jnp.int32, (L, 2 * L), 1)
    first = col < L
    visible = (row < M) | (row >= jnp.where(first, col, col - L))
    low = lax.broadcasted_iota(jnp.int32, (L, LANES), 1) < head_dim - LANES

    def split_pair(a):
        a0, a1, a2 = (a[:, n * LANES:(n + 1) * LANES] for n in range(3))
        zero = jnp.zeros_like(a0)
        return jnp.concatenate([
            jnp.concatenate([a0, jnp.where(low, a1, 0.0), zero], axis=1),
            jnp.concatenate([zero, jnp.where(low, 0.0, a1), a2], axis=1),
        ], axis=0)

    def attention_weights(qkv):
        sc = lax.dot_general(
            qkv[:, 0:pair], split_pair(qkv[:, pair:2 * pair]), _NT,
            preferred_element_type=F32)
        sc = jnp.where(visible, sc * b_scale, MASKED)
        m0 = jnp.max(jnp.where(first, sc, -jnp.inf), axis=1, keepdims=True)
        m1 = jnp.max(jnp.where(first, -jnp.inf, sc), axis=1, keepdims=True)
        e = jnp.exp(sc - jnp.where(first, m0, m1))
        l0 = jnp.sum(jnp.where(first, e, 0.0), axis=1, keepdims=True)
        l1 = jnp.sum(jnp.where(first, 0.0, e), axis=1, keepdims=True)
        return e / jnp.where(first, l0, l1)

    def pair_weights(j):
        return jnp.concatenate([_unpack(wqkv[3 * j + n]) for n in range(3)], axis=1)

    def segment(r0, mem, opening=False):
        h = jnp.concatenate([mem, bx[pl.ds(r0, seg), :].astype(F32)], axis=0)
        qkv, probs, o = {}, {}, {}
        res, done = None, 0
        for t in range(n_pair + n_part):
            if opening and t < len(late_slabs):
                turn_weights(late_slabs[t])
            if t == 0:
                w = pair_weights(0)
                cut = D - LANES
                q = _dot(h[:, :cut], w[:cut, :pair])
                q = _dot(h[:, cut:], w[cut:, :pair]) + q
                qkv[t] = jnp.concatenate([q, _dot(h, w[:, pair:])], axis=1)
            elif t < n_pair:
                qkv[t] = _dot(h, pair_weights(t))
            else:
                upto = n_pair * (t - n_pair + 1) // n_part
                if opening and done == early_pairs:
                    cp_wo_rest.wait()
                part = _dot(
                    jnp.concatenate([o[j] for j in range(done, upto)], axis=1),
                    wo[done * pair:upto * pair, :])
                res = part if res is None else part + res
                done = upto
            j = t - B_LAG
            if 0 <= j < n_pair:
                probs[j] = attention_weights(qkv[j])
            j = t - 2 * B_LAG
            if 0 <= j < n_pair:
                o[j] = _dot(probs[j], split_pair(qkv[j][:, 2 * pair:3 * pair]))
        bout[pl.ds(r0, seg), :] = res[M:].astype(BF16)
        return res[:M]

    cp_bx_rest.start()
    for cp in cp_b_first:
        cp.wait()
    mem = segment(0, bmem[...].astype(F32), opening=True)
    cp_aout.start()
    cp_bout(0, seg).start()

    def b_trip(i, mem):
        @pl.when(i == 1)
        def _():
            cp_bx_rest.wait()

        r0 = pl.multiple_of(seg + i * trip_rows, seg)
        for u in range(B_UNROLL):
            mem = segment(pl.multiple_of(r0 + u * seg, seg), mem)
        cp_bout(r0, trip_rows).start()
        return mem

    lax.fori_loop(0, (S - seg) // trip_rows, b_trip, mem)

    cp_aout.wait()
    cp_bout(0, S).wait()


@functools.partial(jax.jit, static_argnames=("B_seg_len",))
def pallas_concat_heads__sliding_local_dilated__memory_aug_recurrent_mem_tr__prompt_kernel(
    A_x: jax.Array,
    A_wqkv: jax.Array,
    A_wo: jax.Array,
    B_x: jax.Array,
    B_mem0: jax.Array,
    B_Wq: jax.Array,
    B_Wk: jax.Array,
    B_Wv: jax.Array,
    B_Wo: jax.Array,
    B_seg_len: int,
):
    B, S, D = A_x.shape
    _, H, Dh = B_Wq.shape
    M = B_mem0.shape[1]
    seg = int(B_seg_len)
    E = H * Dh
    n_pair = H // 2
    n_tile = D // LANES
    assert B == 1 and B_x.shape == (B, S, D)
    assert D % LANES == 0 and n_tile % 2 == 1
    assert H % 2 == 0 and 2 * Dh == 3 * LANES and 2 * (M + seg) <= LANES
    assert M % 8 == 0 and seg % 16 == 0 and S % seg == 0
    assert (S // seg - 1) % B_UNROLL == 0 and S // seg > 2 * B_UNROLL
    assert S % A_ROWS == 0 and n_pair % (S // A_ROWS) == 0 and n_pair > 2 * B_LAG

    def features_first(w):
        return jnp.transpose(w, (1, 2, 0)).reshape(E, D)

    out = pl.pallas_call(
        functools.partial(_kernel, seg=seg, head_dim=Dh),
        out_shape=jax.ShapeDtypeStruct((S, 2 * D), BF16),
        in_specs=[pl.BlockSpec(memory_space=pl.ANY)] * 9,
        out_specs=pl.BlockSpec(memory_space=pl.ANY),
        scratch_shapes=[
            pltpu.VMEM((S, D), BF16),
            pltpu.VMEM((3, D, D), BF16),
            pltpu.VMEM((D, D), BF16),
            pltpu.VMEM((3, D // 2, D), jnp.int32),
            pltpu.VMEM((D // 2, D), jnp.int32),
            pltpu.VMEM((n_tile, A_HALO + A_ROWS, LANES), F32),
            pltpu.VMEM((n_tile, A_HALO + A_ROWS, LANES), F32),
            pltpu.VMEM((S, D), BF16),
            pltpu.VMEM((S, D), BF16),
            pltpu.VMEM((M, D), BF16),
            pltpu.VMEM((3 * n_pair, 2 * Dh, D), BF16),
            pltpu.VMEM((3 * n_pair, D // 2, 2 * Dh), jnp.int32),
            pltpu.VMEM((E, D), BF16),
            pltpu.VMEM((S, D), BF16),
            pltpu.SemaphoreType.DMA((9 + S // A_ROWS,)),
        ],
        compiler_params=pltpu.CompilerParams(vmem_limit_bytes=110 * 1024 * 1024),
        name="local_and_recurrent_attention",
    )(
        A_x.reshape(S, D), A_wqkv, A_wo,
        B_x.reshape(S, D), B_mem0.reshape(M, D),
        features_first(B_Wq), features_first(B_Wk), features_first(B_Wv),
        B_Wo.reshape(E, D),
    )
    return out.reshape(B, S, 2 * D)
```

```python
import functools

import jax
import jax.numpy as jnp
from jax import lax
import jax.experimental.pallas as pl
import jax.experimental.pallas.tpu as pltpu

F32 = jnp.float32
BF16 = jnp.bfloat16
LANES = 128
MASKED = -1000000000.0
LOG2_E = 1.4426950408889634

A_HEADS = 32
A_WINDOW = 8
A_DILATION = 2
A_HALO = 16
A_ROWS = 256
A_BLOCK = 64
A_GROUP = 16
A_TURNS = (0, 0, 0, 5, 5, 6)
B_UNROLL = 3
B_LAG = 2
WO_EARLY_PARTS = 2

_NT = (((1,), (1,)), ((), ()))


def _pack(w):
    return pltpu.bitcast(w, jnp.int32)


def _unpack(w):
    return pltpu.bitcast(w, BF16)


def _dot(a, b):
    return jnp.dot(a, b, preferred_element_type=F32)


def _kernel(
    ax_hbm, awqkv_hbm, awo_hbm, bx_hbm, bmem_hbm, wq_hbm, wk_hbm, wv_hbm, wo_hbm,
    out_hbm,
    ax, awqkv, awo, awqkv_p, awo_p, kbuf, vbuf, aout,
    bx, bmem, wt, wqkv, wo, bout,
    sems,
    *, seg, head_dim,
):
    S, D = ax.shape
    M = bmem.shape[0]
    L = M + seg
    n_slab = wqkv.shape[0]
    n_pair = n_slab // 3
    pair = 2 * head_dim
    n_trip = S // A_ROWS
    n_tile = D // LANES
    a_dh = D // A_HEADS
    trip_rows = B_UNROLL * seg
    early_rows = seg + trip_rows
    n_part = 2 * B_LAG + 1
    early_pairs = n_pair * WO_EARLY_PARTS // n_part

    def rows_of(src, dst, start, size, sem):
        rows = pl.ds(start, size)
        return pltpu.make_async_copy(src.at[rows], dst.at[rows], sems.at[sem])

    def cp_awqkv(n):
        cols = pl.ds(pl.multiple_of(n * D, D), D)
        return pltpu.make_async_copy(awqkv_hbm.at[:, cols], awqkv.at[n], sems.at[n])

    def cp_slab(j, n, sem):
        feats = pl.ds(pl.multiple_of(j * pair, pair), pair)
        return pltpu.make_async_copy(
            (wq_hbm, wk_hbm, wv_hbm)[n].at[feats], wt.at[3 * j + n], sems.at[sem])

    def turn_weights(slab):
        wqkv[slab] = _pack(wt[slab].T)

    trip_slabs = n_slab // n_trip
    late_slabs = range(n_slab - trip_slabs + 1, n_slab)

    def trip_inputs(i, action):
        action(rows_of(
            ax_hbm, ax, pl.multiple_of(i * A_ROWS, A_ROWS), A_ROWS, 9 + i))

        @pl.when(i > 0)
        def _():
            for k in range(1 - trip_slabs, 0):
                action(cp_slab(i * (trip_slabs // 3) + k // 3, k % 3, 9 + i))

        action(cp_slab(i * (trip_slabs // 3), 0, 9 + i))

    cp_awo = pltpu.make_async_copy(awo_hbm, awo, sems.at[3])
    cp_b_first = [cp_slab(k // 3, k % 3, 4) for k in late_slabs] + [
        pltpu.make_async_copy(bmem_hbm, bmem, sems.at[4]),
        rows_of(bx_hbm, bx, 0, early_rows, 4),
        rows_of(wo_hbm, wo, 0, early_pairs * pair, 4),
    ]
    cp_wo_rest = rows_of(
        wo_hbm, wo, early_pairs * pair, (n_pair - early_pairs) * pair, 5)
    cp_bx_rest = rows_of(bx_hbm, bx, early_rows, S - early_rows, 6)
    cp_aout = pltpu.make_async_copy(aout, out_hbm.at[:, pl.ds(0, D)], sems.at[8])

    def cp_bout(r0, n):
        rows = pl.ds(r0, n)
        return pltpu.make_async_copy(
            bout.at[rows], out_hbm.at[rows, pl.ds(D, D)], sems.at[7])

    cp_awo.start()

    @pl.loop(0, 3)
    def _(n):
        cp_awqkv(n).start()

    @pl.loop(0, n_trip)
    def _(i):
        trip_inputs(i, lambda cp: cp.start())

    for cp in cp_b_first:
        cp.start()

    down = lax.broadcasted_iota(jnp.int32, (LANES, LANES), 0)
    across = lax.broadcasted_iota(jnp.int32, (LANES, LANES), 1)
    shift = A_HEADS.bit_length() - 1

    def source_lane(lane, tile):
        feature = (lane & (A_HEADS - 1)) * a_dh + (lane >> shift) * n_tile + tile
        return feature & (LANES - 1)

    def pick(tiles, residue, tile):
        out = tiles[0]
        for t in range(1, n_tile):
            out = jnp.where(residue == (tile - t * LANES) % n_tile, tiles[t], out)
        return out

    cp_awo.wait()
    residue = lax.broadcasted_iota(jnp.int32, (LANES, D), 0) % n_tile
    tiles = [awo[pl.ds(t * LANES, LANES), :].astype(F32) for t in range(n_tile)]
    for t in range(n_tile):
        awo_p[pl.ds(t * LANES // 2, LANES // 2), :] = _pack(_dot(
            (across == source_lane(down, t)).astype(F32).astype(BF16),
            pick(tiles, residue, t).astype(BF16),
        ).astype(BF16))

    @pl.loop(0, 3)
    def _(n):
        cp_awqkv(n).wait()
        residue = lax.broadcasted_iota(jnp.int32, (D // 2, LANES), 1) % n_tile
        tiles = [
            _pack(awqkv[n, :, t * LANES:(t + 1) * LANES]) for t in range(n_tile)]
        for t in range(n_tile):
            awqkv_p[n, :, t * LANES:(t + 1) * LANES] = _pack(_dot(
                _unpack(pick(tiles, residue, t)),
                (down == source_lane(across, t)).astype(F32).astype(BF16),
            ).astype(BF16))

    cp_wo_rest.start()

    for buf in (kbuf, vbuf):
        buf[:, A_ROWS:, :] = jnp.zeros((n_tile, A_HALO, LANES), F32)

    a_scale = a_dh ** -0.5

    def a_rows(i, block):
        return pl.ds(pl.multiple_of(i * A_ROWS + block * A_BLOCK, A_BLOCK), A_BLOCK)

    def a_project(i, block):
        x = ax[a_rows(i, block), :]
        k = _dot(x, _unpack(awqkv_p[1]))
        q = _dot(x, _unpack(awqkv_p[0]))
        v = _dot(x, _unpack(awqkv_p[2]))
        for buf, val in ((kbuf, k), (vbuf, v)):
            for t in range(n_tile):
                tile = val[:, t * LANES:(t + 1) * LANES]
                if block == 0:
                    buf[t, 0:A_HALO, :] = jnp.where(
                        i == 0, jnp.broadcast_to(tile[0:1], (A_HALO, LANES)),
                        buf[t, A_ROWS:, :])
                buf[t, pl.ds(A_HALO + block * A_BLOCK, A_BLOCK), :] = tile
        return q

    def a_attend(i, block, q_block):
        out = []
        for g0 in range(0, A_BLOCK, A_GROUP):
            q = q_block[g0:g0 + A_GROUP]
            at = block * A_BLOCK + g0

            def window(buf, t, w):
                return buf[t, pl.ds(A_HALO + at - w * A_DILATION, A_GROUP), :]

            logits = []
            for w in range(A_WINDOW):
                z = functools.reduce(jnp.add, [
                    q[:, t * LANES:(t + 1) * LANES] * window(kbuf, t, w)
                    for t in range(n_tile)])
                rot = LANES // 2
                while rot >= A_HEADS:
                    z = z + pltpu.roll(z, rot, 1)
                    rot //= 2
                if w * A_DILATION > at:
                    pos = i * A_ROWS + at + lax.broadcasted_iota(jnp.int32, z.shape, 0)
                    z = jnp.where(pos >= w * A_DILATION, z, MASKED / a_scale)
                logits.append(z)
            top = functools.reduce(jnp.maximum, logits)
            e = [jnp.exp2((z - top) * (a_scale * LOG2_E)) for z in logits]
            inv = 1.0 / functools.reduce(jnp.add, e)
            out.append(jnp.concatenate([
                functools.reduce(
                    jnp.add, [e[w] * window(vbuf, t, w) for w in range(A_WINDOW)]) * inv
                for t in range(n_tile)], axis=1))
        return jnp.concatenate(out, axis=0).astype(BF16)

    @pl.loop(0, n_trip)
    def _(i):
        trip_inputs(i, lambda cp: cp.wait())
        n_block = A_ROWS // A_BLOCK
        q, o = {}, {}
        for t in range(2 * n_block):
            if t < n_block:
                q[t] = a_project(i, t)
            else:
                aout[a_rows(i, t - n_block), :] = _dot(
                    o[t - n_block], _unpack(awo_p[...])).astype(BF16)
            if 1 <= t <= n_block:
                o[t - 1] = a_attend(i, t - 1, q[t - 1])
            for k in range(trip_slabs):
                if A_TURNS[k % len(A_TURNS)] == t:
                    turn_weights(
                        jnp.maximum(i * trip_slabs + k + 1 - trip_slabs, 0))

    b_scale = head_dim ** -0.5
    row = lax.broadcasted_iota(jnp.int32, (L, 2 * L), 0)
    col = lax.broadcasted_iota(jnp.int32, (L, 2 * L), 1)
    first = col < L
    visible = (row < M) | (row >= jnp.where(first, col, col - L))
    low = lax.broadcasted_iota(jnp.int32, (L, LANES), 1) < head_dim - LANES

    def split_pair(a):
        a0, a1, a2 = (a[:, n * LANES:(n + 1) * LANES] for n in range(3))
        zero = jnp.zeros_like(a0)
        return jnp.concatenate([
            jnp.concatenate([a0, jnp.where(low, a1, 0.0), zero], axis=1),
            jnp.concatenate([zero, jnp.where(low, 0.0, a1), a2], axis=1),
        ], axis=0)

    def attention_weights(q, k):
        sc = lax.dot_general(q, split_pair(k), _NT, preferred_element_type=F32)
        sc = jnp.where(visible, sc * b_scale, MASKED)
        m0 = jnp.max(jnp.where(first, sc, -jnp.inf), axis=1, keepdims=True)
        m1 = jnp.max(jnp.where(first, -jnp.inf, sc), axis=1, keepdims=True)
        e = jnp.exp(sc - jnp.where(first, m0, m1))
        l0 = jnp.sum(jnp.where(first, e, 0.0), axis=1, keepdims=True)
        l1 = jnp.sum(jnp.where(first, 0.0, e), axis=1, keepdims=True)
        return e / jnp.where(first, l0, l1)

    def project(j, h):
        w = jnp.concatenate([_unpack(wqkv[3 * j + n]) for n in range(3)], axis=1)
        if j == 0:
            cut = D - LANES
            q = _dot(h[:, :cut], w[:cut, :pair])
            q = _dot(h[:, cut:], w[cut:, :pair]) + q
            kv = _dot(h, w[:, pair:])
        else:
            qkv = _dot(h, w)
            q, kv = qkv[:, :pair], qkv[:, pair:]
        return q, kv[:, :pair], kv[:, pair:]

    def segment(r0, mem, opening=False):
        h = jnp.concatenate([mem, bx[pl.ds(r0, seg), :].astype(F32)], axis=0)
        q, k, v, probs, o = {}, {}, {}, {}, {}
        res, done = None, 0
        for t in range(n_pair + n_part):
            if opening and t < len(late_slabs):
                turn_weights(late_slabs[t])
            if t < n_pair:
                q[t], k[t], v[t] = project(t, h)
            else:
                upto = n_pair * (t - n_pair + 1) // n_part
                if opening and done == early_pairs:
                    cp_wo_rest.wait()
                part = _dot(
                    jnp.concatenate([o[j] for j in range(done, upto)], axis=1),
                    wo[done * pair:upto * pair, :])
                res = part if res is None else part + res
                done = upto
            j = t - B_LAG
            if 0 <= j < n_pair:
                probs[j] = attention_weights(q[j], k[j])
            j = t - 2 * B_LAG
            if 0 <= j < n_pair:
                o[j] = _dot(probs[j], split_pair(v[j]))
        bout[pl.ds(r0, seg), :] = res[M:].astype(BF16)
        return res[:M]

    cp_bx_rest.start()
    for cp in cp_b_first:
        cp.wait()
    mem = segment(0, bmem[...].astype(F32), opening=True)
    cp_aout.start()
    cp_bout(0, seg).start()

    def b_trip(i, mem):
        @pl.when(i == 1)
        def _():
            cp_bx_rest.wait()

        r0 = pl.multiple_of(seg + i * trip_rows, seg)
        for u in range(B_UNROLL):
            mem = segment(pl.multiple_of(r0 + u * seg, seg), mem)
        cp_bout(r0, trip_rows).start()
        return mem

    lax.fori_loop(0, (S - seg) // trip_rows, b_trip, mem)

    cp_aout.wait()
    cp_bout(0, S).wait()


@functools.partial(jax.jit, static_argnames=("B_seg_len",))
def pallas_concat_heads__sliding_local_dilated__memory_aug_recurrent_mem_tr__prompt_kernel(
    A_x: jax.Array,
    A_wqkv: jax.Array,
    A_wo: jax.Array,
    B_x: jax.Array,
    B_mem0: jax.Array,
    B_Wq: jax.Array,
    B_Wk: jax.Array,
    B_Wv: jax.Array,
    B_Wo: jax.Array,
    B_seg_len: int,
):
    B, S, D = A_x.shape
    _, H, Dh = B_Wq.shape
    M = B_mem0.shape[1]
    seg = int(B_seg_len)
    E = H * Dh
    n_pair = H // 2
    n_tile = D // LANES
    assert B == 1 and B_x.shape == (B, S, D)
    assert D % LANES == 0 and n_tile % 2 == 1
    assert H % 2 == 0 and 2 * Dh == 3 * LANES and 2 * (M + seg) <= LANES
    assert M % 8 == 0 and seg % 16 == 0 and S % seg == 0
    assert (S // seg - 1) % B_UNROLL == 0 and S // seg > 2 * B_UNROLL
    assert S % A_ROWS == 0 and n_pair % (S // A_ROWS) == 0 and n_pair > 2 * B_LAG

    def features_first(w):
        return jnp.transpose(w, (1, 2, 0)).reshape(E, D)

    out = pl.pallas_call(
        functools.partial(_kernel, seg=seg, head_dim=Dh),
        out_shape=jax.ShapeDtypeStruct((S, 2 * D), BF16),
        in_specs=[pl.BlockSpec(memory_space=pl.ANY)] * 9,
        out_specs=pl.BlockSpec(memory_space=pl.ANY),
        scratch_shapes=[
            pltpu.VMEM((S, D), BF16),
            pltpu.VMEM((3, D, D), BF16),
            pltpu.VMEM((D, D), BF16),
            pltpu.VMEM((3, D // 2, D), jnp.int32),
            pltpu.VMEM((D // 2, D), jnp.int32),
            pltpu.VMEM((n_tile, A_HALO + A_ROWS, LANES), F32),
            pltpu.VMEM((n_tile, A_HALO + A_ROWS, LANES), F32),
            pltpu.VMEM((S, D), BF16),
            pltpu.VMEM((S, D), BF16),
            pltpu.VMEM((M, D), BF16),
            pltpu.VMEM((3 * n_pair, 2 * Dh, D), BF16),
            pltpu.VMEM((3 * n_pair, D // 2, 2 * Dh), jnp.int32),
            pltpu.VMEM((E, D), BF16),
            pltpu.VMEM((S, D), BF16),
            pltpu.SemaphoreType.DMA((9 + S // A_ROWS,)),
        ],
        compiler_params=pltpu.CompilerParams(vmem_limit_bytes=110 * 1024 * 1024),
        name="local_and_recurrent_attention",
    )(
        A_x.reshape(S, D), A_wqkv, A_wo,
        B_x.reshape(S, D), B_mem0.reshape(M, D),
        features_first(B_Wq), features_first(B_Wk), features_first(B_Wv),
        B_Wo.reshape(E, D),
    )
    return out.reshape(B, S, 2 * D)
```
